```python
import jax
import jax.numpy as jnp

def _softmax(x, axis=-1):
    return jax.nn.softmax(x, axis=axis)
def _gelu(x):
    return jax.nn.gelu(x, approximate=True)
def _silu(x):
    return jax.nn.silu(x)
def _sigmoid(x):
    return jax.nn.sigmoid(x)
def _layernorm(x, axis=-1, eps=1e-5):
    m = jnp.mean(x, axis=axis, keepdims=True)
    v = jnp.var(x, axis=axis, keepdims=True)
    return (x - m) / jnp.sqrt(v + eps)
def _scatter_add(tgt, idx, src, axis=0):
    return tgt.at[idx].add(src)
def _segment_sum(src, seg, n):
    return jax.ops.segment_sum(src, seg, n)
class _Rng:
    def __init__(self, key):
        self._k = key
    def _next(self):
        self._k, sub = jax.random.split(self._k)
        return sub
    def normal(self, shape):
        return jax.random.normal(self._next(), shape, dtype=jnp.bfloat16)
    def randint(self, lo, hi, shape):
        return jax.random.randint(self._next(), shape, lo, hi, dtype=jnp.int32)
    def uniform(self, shape, lo=0.0, hi=1.0):
        return jax.random.uniform(self._next(), shape, jnp.bfloat16, lo, hi)
    def permutation(self, n):
        return jax.random.permutation(self._next(), n)


kernel_name = 'sequential_preLN__sliding_block__glu_gated_glu__prompt'

def _fwd_setup_inputs():
    _rng = _Rng(jax.random.key(int.from_bytes(__import__("os").urandom(4), "little")))
    _w = (lambda a: (lambda t: t.astype(jnp.bfloat16) if jnp.issubdtype(t.dtype, jnp.floating) else t)(jnp.asarray(a)))
    def _A_setup():
        B, S, D = 1, 2048, 512
        return {
            "x": _w((lambda *s: _rng.normal(s) * 0.05)(B, S, D)),
            "wqkv": _w((lambda *s: _rng.normal(s) * 0.05)(D, 3 * D)),
            "wo": _w((lambda *s: _rng.normal(s) * 0.05)(D, D)),
        }
    _A_in = _A_setup()

    def _B_setup():
        B, S, D, F = 1, 2048, 512, 1376
        return {
            "x": _w((lambda *s: _rng.normal(s) * 0.05)(B, S, D)),
            "w_gate": _w((lambda *s: _rng.normal(s) * 0.05)(D, F)),
            "w_up": _w((lambda *s: _rng.normal(s) * 0.05)(D, F)),
            "w_down": _w((lambda *s: _rng.normal(s) * 0.05)(F, D)),
        }
    _B_in = _B_setup()

    return {
        "A_x": _A_in["x"],
        "A_wqkv": _A_in["wqkv"],
        "A_wo": _A_in["wo"],
        "B_x": _B_in["x"],
        "B_w_gate": _B_in["w_gate"],
        "B_w_up": _B_in["w_up"],
        "B_w_down": _B_in["w_down"],
    }

def _fwd_reference(A_x, A_wqkv, A_wo, B_x, B_w_gate, B_w_up, B_w_down):
    def _A_ref(x, wqkv, wo):
        B, S, D = x.shape
        H = 32; Dh = D // H; W = 256
        qkv = (lambda x, *d: x.transpose(*d))((x @ wqkv).reshape(B, S, 3, H, Dh), 2, 0, 3, 1, 4)
        q, k, v = qkv[0], qkv[1], qkv[2]
        scores = jnp.einsum("bhqd,bhkd->bhqk", q, k) * (Dh ** -0.5)
        idx = jnp.arange(S)
        mask = (idx[:, None] - idx[None, :] >= 0) & (idx[:, None] - idx[None, :] < W)
        scores = jnp.where(mask[None, None], scores, -1e9)
        p = _softmax(scores, axis=-1)
        o = jnp.einsum("bhqk,bhkd->bhqd", p, v)
        return (lambda x, *d: x.transpose(*d))(o, 0, 2, 1, 3).reshape(B, S, D) @ wo

    def _B_ref(x, w_gate, w_up, w_down):
        g = jnp.einsum("bsd,df->bsf", x, w_gate)
        u = jnp.einsum("bsd,df->bsf", x, w_up)
        h = _sigmoid(g) * u
        return jnp.einsum("bsf,fd->bsd", h, w_down)

    x = A_x
    h = x + _A_ref(_layernorm(x, axis=-1), A_wqkv, A_wo)
    h2 = h + _B_ref(_layernorm(h, axis=-1), B_w_gate, B_w_up, B_w_down)
    return h2


def setup_inputs():
    _inp = _fwd_setup_inputs()
    _gk = jax.random.fold_in(jax.random.key(int.from_bytes(__import__("os").urandom(4), "little")), 2**31 - 1)
    _shapes = [[1, 2048, 512]]
    _dtypes = ['bfloat16']
    _gks = jax.random.split(_gk, len(_shapes))
    _gs = [jax.random.normal(k, s, dtype=jnp.dtype(d)) * 0.05 for k, s, d in zip(_gks, _shapes, _dtypes)]
    _inp["grad_out"] = _gs[0]
    return _inp

def reference(A_x, A_wqkv, A_wo, B_w_gate, B_w_up, B_w_down, B_x, grad_out):
    _const = dict(B_x=B_x)
    def _f(*_d):
        return _fwd_reference(**{'A_x': _d[0], 'A_wqkv': _d[1], 'A_wo': _d[2], 'B_w_gate': _d[3], 'B_w_up': _d[4], 'B_w_down': _d[5], **_const})
    _out, _vjp = jax.vjp(_f, A_x, A_wqkv, A_wo, B_w_gate, B_w_up, B_w_down)
    _grads = _vjp(grad_out)
    _out0 = jnp.asarray(_out)
    return (_out0, *[jnp.asarray(_g) for _g in _grads])
```

```python
import math

import jax
import jax.numpy as jnp
from jax import lax
import jax.experimental.pallas as pl
import jax.experimental.pallas.tpu as pltpu

S, D, F = 2048, 512, 1376
H, DH = 32, 16
BLK = 128
NB = S // BLK
NG = D // 128
T = 512
NC = S // T
BPC = T // BLK
EPS = 1e-5
LOG2E = math.log2(math.e)
LN2 = math.log(2.0)
F32, BF16 = jnp.float32, jnp.bfloat16


def _nn(a, b):
    return lax.dot_general(a, b, (((1,), (0,)), ((), ())), preferred_element_type=F32)


def _nt(a, b):
    return lax.dot_general(a, b, (((1,), (1,)), ((), ())), preferred_element_type=F32)


def _tn(a, b):
    return lax.dot_general(a, b, (((0,), (0,)), ((), ())), preferred_element_type=F32)


def _ln(x):
    m = jnp.mean(x, axis=-1, keepdims=True)
    xc = x - m
    r = lax.rsqrt(jnp.mean(xc * xc, axis=-1, keepdims=True) + EPS)
    return xc * r, r


def _ln_bwd(dy, xh, r):
    a = jnp.mean(dy, axis=-1, keepdims=True)
    c = jnp.mean(dy * xh, axis=-1, keepdims=True)
    return r * (dy - a - xh * c)


def _pad_head(t, hh):
    parts = []
    if hh > 0:
        parts.append(jnp.zeros((DH * hh, t.shape[1]), t.dtype))
    parts.append(t)
    if hh < 7:
        parts.append(jnp.zeros((DH * (7 - hh), t.shape[1]), t.dtype))
    return jnp.concatenate(parts, axis=0)


def _merge(s, n, tri):
    if n == 3:
        return [jnp.where(tri, s[2 * BLK:], s[:BLK]), s[BLK:2 * BLK]]
    return None


def _split(ps, n, tri):
    z = jnp.zeros_like(ps[0])
    lo = jnp.where(tri, ps[0], z)
    if n == 3:
        return jnp.concatenate([jnp.where(tri, z, ps[0]), ps[1], lo], axis=0)
    if n == 2:
        return jnp.concatenate([ps[1], lo], axis=0)
    return lo


def _cols(ref, c, rows=None):
    if rows is None:
        return jnp.concatenate([ref[c * BPC + i] for i in range(BPC)], axis=1)
    return jnp.concatenate([ref[c * BPC + i, rows, :] for i in range(BPC)], axis=1)


def _put_cols(ref, c, v):
    for i in range(BPC):
        ref[c * BPC + i] = v[:, i * BLK:(i + 1) * BLK]


def _kernel(x_h, wqkv_h, wo_h, wg_h, wu_h, wd_h, g_h,
            out_h, dx_h, dwqkv_h, dwo_h, dwg_h, dwu_h, dwd_h,
            xs, gs, wqkv, wo, wg, wu, wd,
            xnT, qT, kT, vT, kk, vv, oT, linv, pbuf, dhs,
            ostage, dwo_s, dwqkv_s, dwg_s, dwu_s, dwd_s,
            isem, osem):
    def in_copy(i):
        src, dst = ((x_h, xs), (wqkv_h, wqkv), (wo_h, wo), (wg_h, wg), (wu_h, wu),
                    (wd_h, wd), (g_h, gs))[i]
        return pltpu.make_async_copy(src, dst, isem.at[i])

    for i in range(7):
        in_copy(i).start()
    in_copy(0).wait()
    in_copy(1).wait()

    tri = (lax.broadcasted_iota(jnp.int32, (BLK, BLK), 0)
           <= lax.broadcasted_iota(jnp.int32, (BLK, BLK), 1))

    def p1(c, _):
        r0 = pl.multiple_of(c * T, T)
        xh, _r = _ln(xs[pl.ds(r0, T), :].astype(F32))
        xn = xh.astype(BF16)
        _put_cols(xnT, c, xn.T)
        q = (_nn(xn, wqkv[:, 0:D]) * (LOG2E * DH ** -0.5)).astype(BF16)
        _put_cols(qT, c, q.T)
        k = _nn(xn, wqkv[:, D:2 * D]).astype(BF16)
        _put_cols(kT, c, k.T)
        v = _nn(xn, wqkv[:, 2 * D:3 * D]).astype(BF16)
        _put_cols(vT, c, v.T)
        for g in range(NG):
            kk[g, pl.ds(r0, T), :] = k[:, g * 128:(g + 1) * 128]
            vv[g, pl.ds(r0, T), :] = v[:, g * 128:(g + 1) * 128]
        return 0
    lax.fori_loop(0, NC, p1, 0)

    def att_fwd(b, g, n):
        k0 = pl.multiple_of((b - (n - 1)) * BLK, BLK)
        kwin = kk[g, pl.ds(k0, n * BLK), :]
        ones = jnp.ones((DH, n * BLK), BF16)
        for hh in range(8):
            r = pl.ds(pl.multiple_of(g * 128 + hh * DH, DH), DH)
            s = _nn(kwin, _pad_head(qT[b, r, :], hh))
            if n == 3:
                ss = [jnp.where(tri, s[2 * BLK:], s[:BLK]), s[BLK:2 * BLK]]
            else:
                ss = [jnp.where(tri, s[(n - 1) * BLK:], -jnp.inf)] + ([s[:BLK]] if n == 2 else [])
            mx = ss[0] if n == 1 else jnp.maximum(ss[0], ss[1])
            m = jnp.max(mx, axis=0, keepdims=True)
            ps = [jnp.exp2(t - m).astype(BF16) for t in ss]
            for i, p in enumerate(ps):
                pbuf[b, g * 8 + hh, i * BLK:(i + 1) * BLK, :] = p
            vt = jnp.concatenate([vT[b - (n - 1) + i, r, :] for i in range(n)], axis=1)
            o = _nn(jnp.concatenate([vt, ones], axis=0), _split(ps, n, tri))
            li = 1.0 / o[DH:DH + 8]
            oT[b, r, :] = (o[:DH] * jnp.concatenate([li, li], axis=0)).astype(BF16)
            linv[b, g * 8 + hh] = li

    def loop_att(fn):
        lax.fori_loop(0, NG, lambda g, _: fn(0, g, 1), None)
        lax.fori_loop(0, NG, lambda g, _: fn(1, g, 2), None)
        lax.fori_loop(2 * NG, NB * NG, lambda i, _: fn(i // NG, i % NG, 3), None)

    in_copy(2).wait(); in_copy(3).wait(); in_copy(4).wait(); in_copy(5).wait(); in_copy(6).wait()
    loop_att(att_fwd)

    dwo_s[...] = jnp.zeros_like(dwo_s)
    dwg_s[...] = jnp.zeros_like(dwg_s)
    dwu_s[...] = jnp.zeros_like(dwu_s)
    dwd_s[...] = jnp.zeros_like(dwd_s)

    def p3(c, _):
        r0 = pl.multiple_of(c * T, T)
        rows = pl.ds(r0, T)
        ot = _cols(oT, c)
        h = xs[rows, :].astype(F32) + _tn(ot, wo[...])
        hx, rr = _ln(h)
        hn = hx.astype(BF16)
        gate = _nn(hn, wg[...])
        up = _nn(hn, wu[...])
        sg = jax.nn.sigmoid(gate)
        act = (sg * up).astype(BF16)
        ostage[0, rows, :] = (h + _nn(act, wd[...])).astype(BF16)
        go = gs[rows, :]
        da = _nt(go, wd[...])
        du32 = da * sg
        dg = (du32 * up * (1.0 - sg)).astype(BF16)
        du = du32.astype(BF16)
        dhn = _nt(dg, wg[...]) + _nt(du, wu[...])
        hnT = hn.T
        dwg_s[...] += _nn(hnT, dg)
        dwu_s[...] += _nn(hnT, du)
        dwd_s[...] += _tn(go, act)
        dh = go.astype(F32) + _ln_bwd(dhn, hx, rr)
        dhs[rows, :] = dh
        dhb = dh.astype(BF16)
        dwo_s[...] += _nn(ot, dhb)
        return 0
    lax.fori_loop(0, NC, p3, 0)

    wg[...] = dwg_s[...].astype(BF16)
    wu[...] = dwu_s[...].astype(BF16)
    wd[...] = dwd_s[...].T.astype(BF16)
    outs = [pltpu.make_async_copy(ostage.at[0], out_h, osem.at[0]),
            pltpu.make_async_copy(wg, dwg_h, osem.at[1]),
            pltpu.make_async_copy(wu, dwu_h, osem.at[2]),
            pltpu.make_async_copy(wd, dwd_h, osem.at[3])]
    for o_ in outs:
        o_.start()


    def p4(dqT, dkT, dvT):
        dkT[...] = jnp.zeros_like(dkT)
        dvT[...] = jnp.zeros_like(dvT)

        def att_bwd(b, g, n):
            rows = pl.ds(pl.multiple_of(b * BLK, BLK), BLK)
            gr = pl.ds(pl.multiple_of(g * 128, 128), 128)
            doT = _nt(wo[gr, :], dhs[rows, :].astype(BF16))
            k0 = pl.multiple_of((b - (n - 1)) * BLK, BLK)
            vwin = vv[g, pl.ds(k0, n * BLK), :]
            for hh in range(8):
                r = pl.ds(pl.multiple_of(g * 128 + hh * DH, DH), DH)
                li = linv[b, g * 8 + hh]
                do = doT[hh * DH:(hh + 1) * DH] * jnp.concatenate([li, li], axis=0)
                delta = jnp.sum(do * oT[b, r, :].astype(F32), axis=0, keepdims=True)
                do = do.astype(BF16)
                dp = _nn(vwin, _pad_head(do, hh))
                if n == 3:
                    dd = [jnp.where(tri, dp[2 * BLK:], dp[:BLK]), dp[BLK:2 * BLK]]
                else:
                    dd = [dp[(n - 1) * BLK:]] + ([dp[:BLK]] if n == 2 else [])
                ps = [pbuf[b, g * 8 + hh, i * BLK:(i + 1) * BLK, :] for i in range(len(dd))]
                ds = [(p.astype(F32) * (t - delta)).astype(BF16) for p, t in zip(ps, dd)]
                dsc = _split(ds, n, tri)
                kt = jnp.concatenate([kT[b - (n - 1) + i, r, :] for i in range(n)], axis=1)
                dqT[b, r, :] = (_nn(kt, dsc) * DH ** -0.5).astype(BF16)
                dv = _nt(do, _split(ps, n, tri))
                dk = _nt(qT[b, r, :], dsc)
                for i in range(n):
                    dvT[b - (n - 1) + i, r, :] += dv[:, i * BLK:(i + 1) * BLK]
                    dkT[b - (n - 1) + i, r, :] += dk[:, i * BLK:(i + 1) * BLK]
        loop_att(att_bwd)

        outs[0].wait()
        dwqkv_s[...] = jnp.zeros_like(dwqkv_s)

        def p5(c, _):
            rows = pl.ds(pl.multiple_of(c * T, T), T)
            d = jnp.concatenate([_cols(dqT, c), (_cols(dkT, c) * LN2).astype(BF16),
                                 _cols(dvT, c).astype(BF16)], axis=0)
            dxn = _nn(wqkv[...], d).T
            dwqkv_s[...] += _nt(_cols(xnT, c), d)
            xh, rr = _ln(xs[rows, :].astype(F32))
            ostage[0, rows, :] = (dhs[rows, :] + _ln_bwd(dxn, xh, rr)).astype(BF16)
            return 0
        lax.fori_loop(0, NC, p5, 0)

    pl.run_scoped(p4, pltpu.VMEM((NB, D, BLK), BF16), pltpu.VMEM((NB, D, BLK), F32),
                  pltpu.VMEM((NB, D, BLK), F32))
    wqkv[...] = dwqkv_s[...].astype(BF16)
    wo[...] = dwo_s[...].astype(BF16)
    last = [pltpu.make_async_copy(ostage.at[0], dx_h, osem.at[0]),
            pltpu.make_async_copy(wqkv, dwqkv_h, osem.at[4]),
            pltpu.make_async_copy(wo, dwo_h, osem.at[5])]
    for o_ in last:
        o_.start()
    for o_ in outs[1:] + last:
        o_.wait()


@jax.jit
def pallas_sequential_preLN__sliding_block__glu_gated_glu__prompt_kernel(
    A_x, A_wqkv, A_wo, B_x, B_w_gate, B_w_up, B_w_down, grad_out,
):
    V = pltpu.VMEM
    fm = lambda dt: V((NB, D, BLK), dt)
    sds = lambda *s: jax.ShapeDtypeStruct(s, BF16)
    anyspec = pl.BlockSpec(memory_space=pl.ANY)
    outs = pl.pallas_call(
        _kernel,
        in_specs=[anyspec] * 7,
        out_specs=[anyspec] * 7,
        out_shape=[sds(S, D), sds(S, D), sds(D, 3 * D), sds(D, D), sds(D, F), sds(D, F), sds(F, D)],
        scratch_shapes=[
            V((S, D), BF16), V((S, D), BF16), V((D, 3 * D), BF16), V((D, D), BF16),
            V((D, F), BF16), V((D, F), BF16), V((F, D), BF16),
            fm(BF16), fm(BF16), fm(BF16), fm(BF16),
            V((NG, S, 128), BF16), V((NG, S, 128), BF16), fm(BF16),
            V((NB, H, 8, BLK), F32), V((NB, H, 2 * BLK, BLK), BF16), V((S, D), F32),
            V((1, S, D), BF16), V((D, D), F32), V((D, 3 * D), F32),
            V((D, F), F32), V((D, F), F32), V((D, F), F32),
            pltpu.SemaphoreType.DMA((7,)), pltpu.SemaphoreType.DMA((6,)),
        ],
        compiler_params=pltpu.CompilerParams(vmem_limit_bytes=127 * 2 ** 20),
    )(A_x.reshape(S, D), A_wqkv, A_wo, B_w_gate, B_w_up, B_w_down, grad_out.reshape(S, D))
    return (outs[0].reshape(1, S, D), outs[1].reshape(1, S, D), *outs[2:])
```

```python
import math

import jax
import jax.numpy as jnp
from jax import lax
import jax.experimental.pallas as pl
import jax.experimental.pallas.tpu as pltpu

S, D, F = 2048, 512, 1376
H, DH = 32, 16
BLK = 128
NB = S // BLK
HB = BLK // 2
NG = D // 128
T = 256
NC = S // T
BPC = T // BLK
EPS = 1e-5
LA, LC, GU = 4, 2, 4
LOG2E = math.log2(math.e)
LN2 = math.log(2.0)
F32, BF16 = jnp.float32, jnp.bfloat16


def _nn(a, b):
    return lax.dot_general(a, b, (((1,), (0,)), ((), ())), preferred_element_type=F32)


def _nt(a, b):
    return lax.dot_general(a, b, (((1,), (1,)), ((), ())), preferred_element_type=F32)


def _tn(a, b):
    return lax.dot_general(a, b, (((0,), (0,)), ((), ())), preferred_element_type=F32)


def _ln(x):
    m = jnp.mean(x, axis=-1, keepdims=True)
    xc = x - m
    r = lax.rsqrt(jnp.mean(xc * xc, axis=-1, keepdims=True) + EPS)
    return xc * r, r


def _ln_bwd(dy, xh, r):
    a = jnp.mean(dy, axis=-1, keepdims=True)
    c = jnp.mean(dy * xh, axis=-1, keepdims=True)
    return r * (dy - a - xh * c)


def _pad_head(t, hh):
    parts = []
    if hh > 0:
        parts.append(jnp.zeros((DH * hh, t.shape[1]), t.dtype))
    parts.append(t)
    if hh < 7:
        parts.append(jnp.zeros((DH * (7 - hh), t.shape[1]), t.dtype))
    return jnp.concatenate(parts, axis=0)


def _pack(t):
    return pltpu.pack_elementwise([t[:HB], t[HB:]], packed_dtype=BF16)


def _unpack(u):
    return jnp.concatenate([pltpu.unpack_elementwise(u, index=i, packed_dtype=BF16, unpacked_dtype=F32)
                            for i in range(2)], axis=0)


def _deinterleave(k):
    return jnp.concatenate([_unpack(pltpu.bitcast(k[i * BLK:(i + 1) * BLK], jnp.uint32))
                            for i in range(BPC)], axis=0).astype(BF16)


def _split(ps, n, tri_bits):
    lo = ps[0] & tri_bits
    parts = [[lo], [ps[-1], lo], [ps[0] ^ lo, ps[-1], lo]][n - 1]
    return pltpu.bitcast(jnp.concatenate(parts, axis=0), BF16)


def _acc(ref, c, v):
    if c == 0:
        ref[...] = v
    else:
        ref[...] += v


def _cols(ref, c, rows=None):
    if rows is None:
        return jnp.concatenate([ref[c * BPC + i] for i in range(BPC)], axis=1)
    return jnp.concatenate([ref[c * BPC + i, rows, :] for i in range(BPC)], axis=1)


def _put_cols(ref, c, v):
    for i in range(BPC):
        ref[c * BPC + i] = v[:, i * BLK:(i + 1) * BLK]


def _kernel(x_h, wqkv_h, wo_h, wg_h, wu_h, wd_h, g_h,
            out_h, dx_h, dwqkv_h, dwo_h, dwg_h, dwu_h, dwd_h,
            xs, gs, wqkv, wo, wg, wu, wd,
            xnT, qT, kT, vT, kk, vv, oT, linv, pbuf, dhs,
            ostage, dwo_s, dwqkv_s, dwg_s, dwu_s, dwd_s,
            dwo_b, isem, osem, xsem):
    def in_copy(i):
        src, dst = ((x_h, xs), (wqkv_h, wqkv), (wo_h, wo), (wg_h, wg), (wu_h, wu),
                    (wd_h, wd), (g_h, gs))[i]
        return pltpu.make_async_copy(src, dst, isem.at[i])

    def x_copy(c):
        sl = pl.ds(c * T, T)
        return pltpu.make_async_copy(x_h.at[sl], xs.at[sl], xsem.at[c])

    def w_copy(j):
        sl = pl.ds(j * D, D)
        return pltpu.make_async_copy(wqkv_h.at[:, sl], wqkv.at[:, sl], xsem.at[NC + j])

    def o_copy(c, dst):
        sl = pl.ds(c * T, T)
        return pltpu.make_async_copy(ostage.at[0, sl], dst.at[sl], xsem.at[c])

    def w(j):
        if pl_state["c"] == 0:
            w_copy(j).wait()
        return wqkv[:, j * D:(j + 1) * D]
    pl_state = {"c": 0}

    x_copy(0).start()
    for j in range(3):
        w_copy(j).start()
    x_copy(1).start()

    j1 = lax.broadcasted_iota(jnp.int32, (BLK, BLK), 0)
    tri = (jnp.where(j1 < HB, 2 * j1, 2 * j1 - (BLK - 1))
           <= lax.broadcasted_iota(jnp.int32, (BLK, BLK), 1))
    tb = jnp.where(tri, 0xFFFF, 0x0).astype(jnp.uint32)
    tri_bits = tb[:HB] | (tb[HB:] << 16)
    def p1(c, _):
        r0 = c * T
        pl_state["c"] = c
        x_copy(c).wait()
        xh, _r = _ln(xs[pl.ds(r0, T), :].astype(F32))
        xn = xh.astype(BF16)
        _put_cols(xnT, c, xn.T)
        q = (_nn(xn, w(0)) * (LOG2E * DH ** -0.5)).astype(BF16)
        _put_cols(qT, c, q.T)
        k = _nn(xn, w(1)).astype(BF16)
        _put_cols(kT, c, k.T)
        v = _nn(xn, w(2)).astype(BF16)
        _put_cols(vT, c, v.T)
        if c == 0:
            for i in range(2, NC):
                x_copy(i).start()
        if c == 1:
            for i in range(2, 7):
                in_copy(i).start()
        k, v = _deinterleave(k), _deinterleave(v)
        for g in range(NG):
            kk[g, pl.ds(r0, T), :] = k[:, g * 128:(g + 1) * 128]
            vv[g, pl.ds(r0, T), :] = v[:, g * 128:(g + 1) * 128]
        return 0
    with jax.named_scope('p1'):
        [p1(c, 0) for c in range(NC)]

    def att_fwd(b, g, n):
        k0 = pl.multiple_of((b - (n - 1)) * BLK, BLK)
        kwin = [kk[g + j, pl.ds(k0, n * BLK), :] for j in range(GU)]
        ones = jnp.ones((DH, n * BLK), BF16)
        rr = [pl.ds(pl.multiple_of(g * 128 + hh * DH, DH), DH) for hh in range(8 * GU)]

        def st_a(hh):
            return _nn(kwin[hh // 8], _pad_head(qT[b, rr[hh], :], hh % 8))

        def st_b(hh, s):
            if n == 3:
                ss = [jnp.where(tri, s[2 * BLK:], s[:BLK]), s[BLK:2 * BLK]]
            else:
                ss = [jnp.where(tri, s[(n - 1) * BLK:], -jnp.inf)] + ([s[:BLK]] if n == 2 else [])
            mx = ss[0] if n == 1 else jnp.maximum(ss[0], ss[1])
            m = jnp.max(mx, axis=0, keepdims=True)
            ps = [_pack(jnp.exp2(t - m)) for t in ss]
            for i, p in enumerate(ps):
                pbuf[b, g * 8 + hh, i * HB:(i + 1) * HB, :] = p
            return ps

        def st_c(hh, ps):
            r = rr[hh]
            vt = jnp.concatenate([vT[b - (n - 1) + i, r, :] for i in range(n)], axis=1)
            o = _nn(jnp.concatenate([vt, ones], axis=0), _split(ps, n, tri_bits))
            li = 1.0 / o[DH:DH + 8]
            oT[b, r, :] = (o[:DH] * jnp.concatenate([li, li], axis=0)).astype(BF16)
            linv[b, g * 8 + hh] = li
        pipe(st_a, st_b, st_c)

    def pipe(st_a, st_b, st_c):
        sa, sb = {}, {}
        for i in range(-LA, 8 * GU + LC):
            if 0 <= i + LA < 8 * GU:
                sa[i + LA] = st_a(i + LA)
            if 0 <= i < 8 * GU:
                sb[i] = st_b(i, sa.pop(i))
            if 0 <= i - LC < 8 * GU:
                st_c(i - LC, sb.pop(i - LC))

    def loop_att(fn, e=NG):
        lax.fori_loop(0, NG // GU, lambda g, _: fn(0, g * GU, 1), None)
        lax.fori_loop(0, NG // GU, lambda g, _: fn(1, g * GU, 2), None)
        ng = NG // GU
        lax.fori_loop(2 * ng, NB * ng, lambda i, _: fn(i // ng, i % ng * GU, 3), None)

    in_copy(2).wait(); in_copy(3).wait(); in_copy(4).wait(); in_copy(5).wait(); in_copy(6).wait()
    with jax.named_scope('p2'):
        loop_att(att_fwd)


    def p3(c, _):
        r0 = c * T
        rows = pl.ds(r0, T)
        ot = _cols(oT, c)
        h = xs[rows, :].astype(F32) + _tn(ot, wo[...])
        hx, rr = _ln(h)
        hn = hx.astype(BF16)
        gate = _nt(hn, wg[...])
        up = _nt(hn, wu[...])
        sg = jax.nn.sigmoid(gate)
        act = (sg * up).astype(BF16)
        ostage[0, rows, :] = (h + _nn(act, wd[...])).astype(BF16)
        go = gs[rows, :]
        da = _nt(go, wd[...])
        du32 = da * sg
        dg = (du32 * up * (1.0 - sg)).astype(BF16)
        du = du32.astype(BF16)
        dhn = _nn(dg, wg[...]) + _nn(du, wu[...])
        hnT = hn.T
        _acc(dwg_s, c, _nn(hnT, dg))
        _acc(dwu_s, c, _nn(hnT, du))
        _acc(dwd_s, c, _tn(go, act))
        dh = go.astype(F32) + _ln_bwd(dhn, hx, rr)
        dhs[rows, :] = dh
        dhb = dh.astype(BF16)
        _acc(dwo_s, c, _nn(ot, dhb))
        o_copy(c, out_h).start()
        return 0
    with jax.named_scope('p3'):
        [p3(c, 0) for c in range(NC)]

    wg[...] = dwg_s[...].T.astype(BF16)
    wu[...] = dwu_s[...].T.astype(BF16)
    wd[...] = dwd_s[...].T.astype(BF16)
    dwo_b[...] = dwo_s[...].astype(BF16)
    outs = [pltpu.make_async_copy(dwo_b, dwo_h, osem.at[5]),
            pltpu.make_async_copy(wg, dwg_h, osem.at[1]),
            pltpu.make_async_copy(wu, dwu_h, osem.at[2]),
            pltpu.make_async_copy(wd, dwd_h, osem.at[3])]
    for o_ in outs:
        o_.start()


    def p4(dqT, dkT, dvT):
        dkT[...] = jnp.zeros_like(dkT)
        dvT[...] = jnp.zeros_like(dvT)

        def att_bwd(b, g, n):
            rows = pl.ds(pl.multiple_of(b * BLK, BLK), BLK)
            gr = pl.ds(pl.multiple_of(g * 128, 128), 128 * GU)
            doT = _nt(wo[gr, :], dhs[rows, :].astype(BF16))
            k0 = pl.multiple_of((b - (n - 1)) * BLK, BLK)
            vwin = [vv[g + j, pl.ds(k0, n * BLK), :] for j in range(GU)]
            rr = [pl.ds(pl.multiple_of(g * 128 + hh * DH, DH), DH) for hh in range(8 * GU)]

            def st_a(hh):
                li = linv[b, g * 8 + hh]
                do = doT[hh * DH:(hh + 1) * DH] * jnp.concatenate([li, li], axis=0)
                delta = jnp.sum(do * oT[b, rr[hh], :].astype(F32), axis=0, keepdims=True)
                do = do.astype(BF16)
                return do, delta, _nn(vwin[hh // 8], _pad_head(do, hh % 8))

            def st_b(hh, a):
                do, delta, dp = a
                if n == 3:
                    dd = [jnp.where(tri, dp[2 * BLK:], dp[:BLK]), dp[BLK:2 * BLK]]
                else:
                    dd = [dp[(n - 1) * BLK:]] + ([dp[:BLK]] if n == 2 else [])
                ps = [pbuf[b, g * 8 + hh, i * HB:(i + 1) * HB, :] for i in range(len(dd))]
                ds = [_pack(_unpack(p) * (t - delta)) for p, t in zip(ps, dd)]
                return ds, _nt(do, _split(ps, n, tri_bits))

            def st_c(hh, a):
                ds, dv = a
                r = rr[hh]
                dsc = _split(ds, n, tri_bits)
                kt = jnp.concatenate([kT[b - (n - 1) + i, r, :] for i in range(n)], axis=1)
                dqT[b, r, :] = (_nn(kt, dsc) * DH ** -0.5).astype(BF16)
                dk = _nt(qT[b, r, :], dsc)
                for i in range(n):
                    dvT[b - (n - 1) + i, r, :] += dv[:, i * BLK:(i + 1) * BLK]
                    dkT[b - (n - 1) + i, r, :] += dk[:, i * BLK:(i + 1) * BLK]
            pipe(st_a, st_b, st_c)
        with jax.named_scope('p4'):
            loop_att(att_bwd)

        for c in range(NC):
            o_copy(c, out_h).wait()

        def p5(c, _):
            rows = pl.ds(c * T, T)
            d = jnp.concatenate([_cols(dqT, c), (_cols(dkT, c) * LN2).astype(BF16),
                                 _cols(dvT, c).astype(BF16)], axis=0)
            dxn = _nn(wqkv[...], d).T
            _acc(dwqkv_s, c, _nt(_cols(xnT, c), d))
            xh, rr = _ln(xs[rows, :].astype(F32))
            ostage[0, rows, :] = (dhs[rows, :] + _ln_bwd(dxn, xh, rr)).astype(BF16)
            o_copy(c, dx_h).start()
            return 0
        with jax.named_scope('p5'):
            [p5(c, 0) for c in range(NC)]

    pl.run_scoped(p4, pltpu.VMEM((NB, D, BLK), BF16), pltpu.VMEM((NB, D, BLK), F32),
                  pltpu.VMEM((NB, D, BLK), F32))
    wqkv[...] = dwqkv_s[...].astype(BF16)
    last = [o_copy(c, dx_h) for c in range(NC)]
    last += [
            pltpu.make_async_copy(wqkv, dwqkv_h, osem.at[4])]
    for o_ in last[-1:]:
        o_.start()
    for o_ in outs + last:
        o_.wait()


@jax.jit
def pallas_sequential_preLN__sliding_block__glu_gated_glu__prompt_kernel(
    A_x, A_wqkv, A_wo, B_x, B_w_gate, B_w_up, B_w_down, grad_out,
):
    V = pltpu.VMEM
    fm = lambda dt: V((NB, D, BLK), dt)
    sds = lambda *s: jax.ShapeDtypeStruct(s, BF16)
    anyspec = pl.BlockSpec(memory_space=pl.ANY)
    outs = pl.pallas_call(
        _kernel,
        in_specs=[anyspec] * 7,
        out_specs=[anyspec] * 7,
        out_shape=[sds(S, D), sds(S, D), sds(D, 3 * D), sds(D, D), sds(F, D), sds(F, D), sds(F, D)],
        scratch_shapes=[
            V((S, D), BF16), V((S, D), BF16), V((D, 3 * D), BF16), V((D, D), BF16),
            V((F, D), BF16), V((F, D), BF16), V((F, D), BF16),
            fm(BF16), fm(BF16), fm(BF16), fm(BF16),
            V((NG, S, 128), BF16), V((NG, S, 128), BF16), fm(BF16),
            V((NB, H, 8, BLK), F32), V((NB, H, BLK, BLK), jnp.uint32), V((S, D), F32),
            V((1, S, D), BF16), V((D, D), F32), V((D, 3 * D), F32),
            V((D, F), F32), V((D, F), F32), V((D, F), F32),
            V((D, D), BF16), pltpu.SemaphoreType.DMA((7,)), pltpu.SemaphoreType.DMA((6,)),
            pltpu.SemaphoreType.DMA((NC + 3,)),
        ],
        compiler_params=pltpu.CompilerParams(vmem_limit_bytes=127 * 2 ** 20),
    )(A_x.reshape(S, D), A_wqkv, A_wo, B_w_gate.T, B_w_up.T, B_w_down, grad_out.reshape(S, D))
    return (outs[0].reshape(1, S, D), outs[1].reshape(1, S, D), outs[2], outs[3], outs[4].T, outs[5].T, outs[6])
```
